```python
import os as _os
_os.environ.setdefault("JAX_PLATFORMS", "cpu")
import jax
import jax.numpy as jnp

def _softmax(x, axis=-1):
    return jax.nn.softmax(x, axis=axis)
def _gelu(x):
    return jax.nn.gelu(x, approximate=True)
def _silu(x):
    return jax.nn.silu(x)
def _sigmoid(x):
    return jax.nn.sigmoid(x)
def _layernorm(x, axis=-1, eps=1e-5):
    m = jnp.mean(x, axis=axis, keepdims=True)
    v = jnp.var(x, axis=axis, keepdims=True)
    return (x - m) / jnp.sqrt(v + eps)
def _scatter_add(tgt, idx, src, axis=0):
    return tgt.at[idx].add(src)
def _segment_sum(src, seg, n):
    return jax.ops.segment_sum(src, seg, n)
class _Rng:
    def __init__(self, key):
        self._k = key
    def _next(self):
        self._k, sub = jax.random.split(self._k)
        return sub
    def normal(self, shape):
        return jax.random.normal(self._next(), shape, dtype=jnp.bfloat16)
    def randint(self, lo, hi, shape):
        return jax.random.randint(self._next(), shape, lo, hi, dtype=jnp.int32)
    def uniform(self, shape, lo=0.0, hi=1.0):
        return jax.random.uniform(self._next(), shape, jnp.bfloat16, lo, hi)
    def permutation(self, n):
        return jax.random.permutation(self._next(), n)


kernel_name = 'concat_heads__sliding_block_cached__compressed_kv_cla__decode'

def setup_inputs():
    _rng = _Rng(jax.random.key(int.from_bytes(__import__("os").urandom(4), "little")))
    _w = (lambda a: (lambda t: t.astype(jnp.bfloat16) if jnp.issubdtype(t.dtype, jnp.floating) else t)(jnp.asarray(a)))
    def _A_setup():
        B, Sq, D = 1, 1, 512
        Hq, Hkv, Sk, Dh = 32, 32, 4096, 128
        assert Hq % Hkv == 0, (Hq, Hkv)
        return {
            "x": _w((lambda *s: _rng.normal(s) * 0.8)(B, Sq, D)),
            "k_cache": _w((lambda *s: _rng.normal(s) * 0.8)(B, Hkv, Sk, Dh)),
            "v_cache": _w((lambda *s: _rng.normal(s) * 0.05)(B, Hkv, Sk, Dh)),
            "wq": _w((lambda *s: _rng.normal(s) * 0.8)(D, Hq * Dh) * (D ** -0.5)),
            "wo": _w((lambda *s: _rng.normal(s) * 0.05)(Hq * Dh, D) * ((Hq * Dh) ** -0.5)),
        }
    _A_in = _A_setup()

    def _B_setup():
        B, H, Sq, Sk, D, M = 1, 32, 1, 4096, 128, 512
        Dc = 4 * D
        return {
            "x": _w((lambda *s: _rng.normal(s) * 1.6)(B, Sq, M)),
            "c_kv": _w((lambda *s: _rng.normal(s) * 0.1)(B, Sk, Dc)),
            "w_q": _w((lambda *s: _rng.normal(s) * 1.6)(M, H, D) * (M ** -0.5)),
            "w_uk": _w((lambda *s: _rng.normal(s) * 1.6)(Dc, H, D) * (Dc ** -0.5)),
            "w_uv": _w((lambda *s: _rng.normal(s) * 0.1)(Dc, H, D) * (Dc ** -0.5)),
            "w_o": _w((lambda *s: _rng.normal(s) * 0.1)(H, D, M) * ((H * D) ** -0.5)),
        }
    _B_in = _B_setup()

    return {
        "A_x": _A_in["x"],
        "A_k_cache": _A_in["k_cache"],
        "A_v_cache": _A_in["v_cache"],
        "A_wq": _A_in["wq"],
        "A_wo": _A_in["wo"],
        "B_x": _B_in["x"],
        "B_c_kv": _B_in["c_kv"],
        "B_w_q": _B_in["w_q"],
        "B_w_uk": _B_in["w_uk"],
        "B_w_uv": _B_in["w_uv"],
        "B_w_o": _B_in["w_o"],
    }

def reference(A_x, A_k_cache, A_v_cache, A_wq, A_wo, B_x, B_c_kv, B_w_q, B_w_uk, B_w_uv, B_w_o):
    def _A_ref(x, k_cache, v_cache, wq, wo):
        B, Sq, D = x.shape
        Hq, Dh = 32, 128
        Hkv, Sk = k_cache.shape[1], k_cache.shape[2]
        W = min(4096, max(256, Sk // 4))
        rep = Hq // Hkv
        q = (lambda x, *d: x.transpose(*d))((x @ wq).reshape(B, Sq, Hq, Dh), 0, 2, 1, 3)
        k = jnp.repeat(k_cache[:, :, Sk - W:, :], rep, axis=1)
        v = jnp.repeat(v_cache[:, :, Sk - W:, :], rep, axis=1)
        scores = jnp.einsum("bhqd,bhkd->bhqk", q, k) * (Dh ** -0.5)
        p = _softmax(scores, axis=-1)
        o = jnp.einsum("bhqk,bhkd->bhqd", p, v)
        return (lambda x, *d: x.transpose(*d))(o, 0, 2, 1, 3).reshape(B, Sq, Hq * Dh) @ wo

    def _B_ref(x, c_kv, w_q, w_uk, w_uv, w_o):
        B, Sq, M = x.shape[0], x.shape[1], x.shape[2]
        Sk = c_kv.shape[1]
        H, D = w_q.shape[1], w_q.shape[2]
        q = jnp.einsum("bqm,mhd->bhqd", x, w_q)
        k = jnp.einsum("bkc,chd->bhkd", c_kv, w_uk)
        v = jnp.einsum("bkc,chd->bhkd", c_kv, w_uv)
        scores = jnp.einsum("bhqd,bhkd->bhqk", q, k) * (D ** -0.5)
        off = Sk - Sq
        qi = jnp.arange(Sq)[:, None]
        kj = jnp.arange(Sk)[None, :]
        cmask = kj <= (qi + off)
        scores = jnp.where(cmask[None, None], scores, -1e9)
        p = _softmax(scores, axis=-1)
        ctx = jnp.einsum("bhqk,bhkd->bhqd", p, v)
        return jnp.einsum("bhqd,hdm->bqm", ctx, w_o)

    a = _A_ref(A_x, A_k_cache, A_v_cache, A_wq, A_wo)
    b = _B_ref(B_x, B_c_kv, B_w_q, B_w_uk, B_w_uv, B_w_o)
    return jnp.concatenate([a, b], axis=-1)
```

```python
import jax
import jax.numpy as jnp
from jax import lax
import jax.experimental.pallas as pl
import jax.experimental.pallas.tpu as pltpu

_NN = (((1,), (0,)), ((), ()))
_NT = (((1,), (1,)), ((), ()))
_BF = jnp.bfloat16
_F32 = jnp.float32


def _dot(a, b, dims=_NN):
    return lax.dot_general(a, b, dims, preferred_element_type=_F32)


def _make_kernel(H, DH, SK, W, D, DC, wo_split):
    HD = H * DH
    NB = DC // 128
    BLK = 128 * H
    scale = DH ** -0.5

    def kernel(ax_hbm, k_hbm, v_hbm, wq_hbm, wo_hbm, bx_hbm, ckv_hbm, bwq_hbm,
               wuk_hbm, wuv_hbm, bwo_hbm, o_ref,
               ax_v, bx_v, k_v, v_v, wq_v, wo_v, ckv_v, bwq_v, wuk_v, wuv_v,
               bwo_v, rexp_v, exp_v, sems):
        copies = []

        def add(src, dst, s):
            c = pltpu.make_async_copy(src, dst, sems.at[s])
            c.start()
            return c

        c_bx = add(bx_hbm, bx_v, 0)
        c_ax = add(ax_hbm, ax_v, 0)
        c_bwq = add(bwq_hbm, bwq_v, 1)
        c_wuk = add(wuk_hbm, wuk_v, 2)
        c_ckv = add(ckv_hbm.at[0], ckv_v, 3)
        c_wq = add(wq_hbm, wq_v, 4)
        c_k = add(k_hbm.at[0, :, pl.ds(SK - W, W), :], k_v, 5)
        c_v = add(v_hbm.at[0, :, pl.ds(SK - W, W), :], v_v, 6)
        c_wuv = add(wuv_hbm, wuv_v, 7)
        c_wo = add(wo_hbm, wo_v, 8)
        c_bwo = []
        r = 0
        for i, n in enumerate(wo_split):
            c_bwo.append(add(bwo_hbm.at[pl.ds(r, n)], bwo_v.at[pl.ds(r, n)], 9 + i))
            r += n

        rows = lax.broadcasted_iota(jnp.int32, (128, BLK), 0)
        cols = lax.broadcasted_iota(jnp.int32, (128, BLK), 1)
        rexp_v[...] = jnp.where(cols // H == rows, 1.0, 0.0).astype(_BF)

        hmask = (lax.broadcasted_iota(jnp.int32, (H, BLK), 1) % H
                 == lax.broadcasted_iota(jnp.int32, (H, BLK), 0))

        def expand(vals):
            for b in range(NB):
                e = _dot(vals[:, b * 128:(b + 1) * 128], rexp_v[...])
                exp_v[b] = jnp.where(hmask, e, 0.0).astype(_BF)

        def contract(w_v):
            acc = _dot(exp_v[0], w_v[0:BLK, :])
            for b in range(1, NB):
                acc += _dot(exp_v[b], w_v[b * BLK:(b + 1) * BLK, :])
            return acc

        def flatten(t):
            r8 = lax.broadcasted_iota(jnp.int32, (8, DH), 0)
            parts = []
            for h in range(H):
                g = h // 8
                parts.append(jnp.where(r8 == h % 8, t[g * 8:(g + 1) * 8, :], 0.0))
            flat = jnp.sum(jnp.concatenate(parts, axis=1), axis=0, keepdims=True)
            return jnp.broadcast_to(flat, (8, HD)).astype(_BF)

        c_bx.wait()
        c_ax.wait()
        expand(jnp.broadcast_to(bx_v[0], (H, D)))
        c_bwq.wait()
        qb = contract(bwq_v).astype(_BF)

        c_wuk.wait()
        qa = []
        for b in range(NB):
            z = _dot(qb, wuk_v[b * BLK:(b + 1) * BLK, :], _NT)
            z = jnp.where(hmask, z, 0.0).astype(_BF)
            qa.append(_dot(z, rexp_v[...], _NT))
        qabs = jnp.concatenate(qa, axis=1).astype(_BF)

        c_ckv.wait()
        s = _dot(qabs, ckv_v[...], _NT) * scale
        m = jnp.max(s, axis=1, keepdims=True)
        p = jnp.exp(s - m)
        l = jnp.sum(p, axis=1, keepdims=True)
        lat = _dot(p.astype(_BF), ckv_v[...]) / l
        expand(lat.astype(_BF))

        c_wq.wait()
        q8 = _dot(jnp.broadcast_to(ax_v[0], (8, D)), wq_v[...])
        r8 = lax.broadcasted_iota(jnp.int32, (8, DH), 0)

        c_k.wait()
        ps = []
        ls = []
        for g in range(H // 8):
            sg = None
            for j in range(8):
                h = g * 8 + j
                qm = jnp.where(r8 == j, q8[:, h * DH:(h + 1) * DH], 0.0).astype(_BF)
                t = _dot(qm, k_v[h], _NT)
                sg = t if sg is None else sg + t
            sg = sg * scale
            mg = jnp.max(sg, axis=1, keepdims=True)
            pg = jnp.exp(sg - mg)
            ls.append(jnp.sum(pg, axis=1, keepdims=True))
            ps.append(pg.astype(_BF))

        c_v.wait()
        os_ = []
        for g in range(H // 8):
            og = jnp.zeros((8, DH), _F32)
            for j in range(8):
                h = g * 8 + j
                og = jnp.where(r8 == j, _dot(ps[g], v_v[h]), og)
            os_.append(og / ls[g])
        oa = flatten(jnp.concatenate(os_, axis=0))

        c_wuv.wait()
        ob = flatten(contract(wuv_v))

        c_wo.wait()
        o_ref[0, :, 0:D] = _dot(oa, wo_v[...])[0:1, :].astype(o_ref.dtype)
        acc = None
        r = 0
        for i, n in enumerate(wo_split):
            c_bwo[i].wait()
            t = _dot(ob[:, r:r + n], bwo_v[r:r + n, :])
            acc = t if acc is None else acc + t
            r += n
        o_ref[0, :, D:2 * D] = acc[0:1, :].astype(o_ref.dtype)

    return kernel


_WO_SPLIT = (2048, 1024, 512, 256, 128, 128)


@jax.jit
def pallas_concat_heads__sliding_block_cached__compressed_kv_cla__decode_kernel(
    A_x, A_k_cache, A_v_cache, A_wq, A_wo, B_x, B_c_kv, B_w_q, B_w_uk, B_w_uv, B_w_o,
):
    wo_split = _WO_SPLIT
    _, H, SK, DH = A_k_cache.shape
    D = A_x.shape[-1]
    DC = B_c_kv.shape[-1]
    W = min(4096, max(256, SK // 4))
    HD = H * DH
    kernel = _make_kernel(H, DH, SK, W, D, DC, wo_split)
    anyspec = pl.BlockSpec(memory_space=pl.ANY)
    scratch = [
        pltpu.VMEM((1, 1, D), _BF), pltpu.VMEM((1, 1, D), _BF),
        pltpu.VMEM((H, W, DH), _BF), pltpu.VMEM((H, W, DH), _BF),
        pltpu.VMEM((D, HD), _BF), pltpu.VMEM((HD, D), _BF),
        pltpu.VMEM((SK, DC), _BF),
        pltpu.VMEM((D * H, DH), _BF), pltpu.VMEM((DC * H, DH), _BF),
        pltpu.VMEM((DC * H, DH), _BF), pltpu.VMEM((HD, D), _BF),
        pltpu.VMEM((128, 128 * H), _BF),
        pltpu.VMEM((DC // 128, H, 128 * H), _BF),
        pltpu.SemaphoreType.DMA((9 + len(wo_split),)),
    ]
    return pl.pallas_call(
        kernel,
        out_shape=jax.ShapeDtypeStruct((1, 1, 2 * D), _BF),
        in_specs=[anyspec] * 11,
        out_specs=pl.BlockSpec(memory_space=pltpu.VMEM),
        scratch_shapes=scratch,
        compiler_params=pltpu.CompilerParams(
            vmem_limit_bytes=96 * 1024 * 1024,
            disable_semaphore_checks=True),
    )(A_x, A_k_cache, A_v_cache, A_wq, A_wo, B_x, B_c_kv,
      B_w_q.reshape(D * H, DH), B_w_uk.reshape(DC * H, DH),
      B_w_uv.reshape(DC * H, DH), B_w_o.reshape(HD, D))
```

```python
import jax
import jax.numpy as jnp
from jax import lax
import jax.experimental.pallas as pl
import jax.experimental.pallas.tpu as pltpu

_NN = (((1,), (0,)), ((), ()))
_NT = (((1,), (1,)), ((), ()))
_BF = jnp.bfloat16
_F32 = jnp.float32

H, DH, SK, W, D, DC = 32, 128, 4096, 1024, 512, 512
HD = H * DH
NB = 4
BLK = 128 * H
NR = 32


def _dot(a, b, dims=_NN):
    return lax.dot_general(a, b, dims, preferred_element_type=_F32)


def _mo(x, m):
    return x if isinstance(x, int) else pl.multiple_of(x, m)


def _make_kernel(groups, sched, early, dA, dB, prefix, vpu_tail):
    scale = DH ** -0.5
    nG = len(groups)

    def kernel(ax_hbm, k_hbm, v_hbm, wq_hbm, wo_hbm, bx_hbm, ckv_hbm, bwq_hbm,
               wuk_hbm, wuv_hbm, bwo_hbm, o_ref,
               ax_v, bx_v, k_v, v_v, wq_v, wo_v, ckv_v, bwq_v, wuk_v, wuv_v,
               bwo_v, rexp_v, exp_v, sems):
        S_X, S_BWQ, S_WQ, S_WUK, S_CKV, S_K, S_V, S_WUV, S_O = range(9)

        def cp(src, dst, sem):
            return pltpu.make_async_copy(src, dst, sems.at[sem])

        def narrow(hbm, vm, j, sem):
            dr = dB * 8

            def mk(i):
                if isinstance(i, int) and i == 0 and j == 0 and dr:
                    a, b = pl.ds(0, 128 - dr), pl.ds(NB * BLK - dr, dr)
                    return [cp(hbm.at[a], vm.at[a], sem), cp(hbm.at[b], vm.at[b], sem)]
                sl = pl.ds(_mo((j * NR + i) * 128 - dr, 8), 128)
                return [cp(hbm.at[sl], vm.at[sl], sem)]
            return mk

        def wide(hbm, vm, j, sem):
            def mk(i):
                sl = pl.ds(_mo(i * 32, 32), 32)
                return [cp(hbm.at[j, sl, :], vm.at[j, sl, :], sem)]
            return mk

        def wq_stream(j):
            def mk(i):
                r = pl.ds(_mo((i >> 1) * 8, 8), 8)
                c = pl.ds(_mo((i & 1) * (HD // 2), HD // 2), HD // 2)
                return [cp(wq_hbm.at[j, r, c], wq_v.at[j, r, c], S_WQ)]
            return mk

        def kv_stream(hbm, vm, s, sem):
            dr = dA * 8

            def mk(i):
                h = 4 * s + (i >> 3)
                if isinstance(i, int) and i % 8 == 0 and dr:
                    return [cp(hbm.at[0, h, pl.ds(SK - W, 128 - dr), :],
                               vm.at[h, pl.ds(0, 128 - dr), :], sem),
                            cp(hbm.at[0, h, pl.ds(SK - dr, dr), :],
                               vm.at[h, pl.ds(W - dr, dr), :], sem)]
                r = _mo((i & 7) * 128 - dr, 8)
                return [cp(hbm.at[0, h, pl.ds(SK - W + r, 128), :],
                           vm.at[h, pl.ds(r, 128), :], sem)]
            return mk

        def interleave(a, b):
            return [x for t in zip(a, b) for x in t]

        def issue(streams, r0, r1, peel=NR, thread=None):
            def one(i):
                for s, mk in enumerate(streams):
                    for c in mk(i):
                        c.start(priority=(s + 1) % 2 if thread is None else thread)

            def body(i, c):
                one(i)
                return c
            i = r0
            while i < r1:
                if i % peel == 0:
                    one(i)
                    i += 1
                    continue
                e = min(r1, (i // peel + 1) * peel)
                lax.fori_loop(i, e, body, 0)
                i = e

        def wait_all(vm, sem):
            pltpu.make_async_copy(vm, vm, sems.at[sem]).wait()

        slot1 = interleave([narrow(bwq_hbm, bwq_v, j, S_BWQ) for j in range(NB)],
                           [wq_stream(j) for j in range(NB)])
        slot2 = interleave([narrow(wuk_hbm, wuk_v, j, S_WUK) for j in range(NB)],
                           [wide(ckv_hbm, ckv_v, j, S_CKV) for j in range(NB)])
        slot3 = [kv_stream(k_hbm, k_v, s, S_K) for s in range(8)]
        slot4 = ([kv_stream(v_hbm, v_v, s, S_V) for s in range(8)]
                 + [narrow(wuv_hbm, wuv_v, j, S_WUV) for j in range(NB)])

        def slot5(g):
            return interleave([wide(wo_hbm, wo_v, j, S_O + g) for j in range(NB)],
                              [wide(bwo_hbm, bwo_v, j, S_O + nG + g) for j in range(NB)])

        c_bx = cp(bx_hbm, bx_v, S_X)
        c_ax = cp(ax_hbm, ax_v, S_X)
        if prefix:
            issue(slot1, 0, prefix, thread=1)
        c_bx.start()
        c_ax.start()
        issue(slot1, prefix, 10)

        def hmask():
            return (lax.broadcasted_iota(jnp.int32, (H, BLK), 1) % H
                    == lax.broadcasted_iota(jnp.int32, (H, BLK), 0))
        r8 = lax.broadcasted_iota(jnp.int32, (8, DH), 0)

        def expand(vals):
            hm = hmask()
            for b in range(NB):
                e = _dot(vals[:, b * 128:(b + 1) * 128], rexp_v[...])
                exp_v[b] = jnp.where(hm, e, 0.0).astype(_BF)

        def contract(w_v):
            acc = _dot(exp_v[0], w_v[0:BLK, :])
            for b in range(1, NB):
                acc += _dot(exp_v[b], w_v[b * BLK:(b + 1) * BLK, :])
            return acc

        def flatten(t):
            parts = []
            for h in range(H):
                g = h // 8
                parts.append(jnp.where(r8 == h % 8, t[g * 8:(g + 1) * 8, :], 0.0))
            flat = jnp.sum(jnp.concatenate(parts, axis=1), axis=0, keepdims=True)
            return jnp.broadcast_to(flat, (8, HD)).astype(_BF)

        rows = lax.broadcasted_iota(jnp.int32, (128, BLK), 0)
        cols = lax.broadcasted_iota(jnp.int32, (128, BLK), 1)
        rexp_v[...] = jnp.where(cols // H == rows, 1.0, 0.0).astype(_BF)
        issue(slot1, 10, 20)
        c_bx.wait()
        c_ax.wait()
        expand(jnp.broadcast_to(bx_v[0], (H, D)))
        issue(slot1, 20, NR)

        issue(slot2, 0, 12)
        wait_all(bwq_v, S_BWQ)
        qb = contract(bwq_v).astype(_BF)
        issue(slot2, 12, 20)
        wait_all(wq_v, S_WQ)
        xa = jnp.broadcast_to(ax_v[0], (8, D))
        q8 = _dot(xa[:, 0:128], wq_v[0])
        for j in range(1, NB):
            q8 += _dot(xa[:, j * 128:(j + 1) * 128], wq_v[j])
        issue(slot2, 20, NR)

        issue(slot3, 0, 11, 8)
        wait_all(wuk_v, S_WUK)
        qa = []
        for b in range(NB):
            z = _dot(qb, wuk_v[b * BLK:(b + 1) * BLK, :], _NT)
            z = jnp.where(hmask(), z, 0.0).astype(_BF)
            qa.append(_dot(z, rexp_v[...], _NT))
            if b == 1:
                issue(slot3, 11, 16, 8)
        qabs = jnp.concatenate(qa, axis=1).astype(_BF)
        issue(slot3, 16, 21, 8)
        wait_all(ckv_v, S_CKV)
        s = jnp.concatenate([_dot(qabs, ckv_v[j], _NT) for j in range(NB)], axis=1) * scale
        m = jnp.max(s, axis=1, keepdims=True)
        p = jnp.exp(s - m)
        l = jnp.sum(p, axis=1, keepdims=True)
        p = p.astype(_BF)
        issue(slot3, 21, 27, 8)
        lat = _dot(p[:, 0:1024], ckv_v[0])
        for j in range(1, NB):
            lat += _dot(p[:, j * 1024:(j + 1) * 1024], ckv_v[j])
        lat = lat / l
        expand(lat.astype(_BF))
        issue(slot3, 27, NR, 8)

        issue(slot4, 0, 8, 8)
        wait_all(k_v, S_K)
        ps = []
        ls = []
        cuts = (8, 16, 20, 24, 32)
        for g in range(H // 8):
            sg = None
            for j in range(8):
                h = g * 8 + j
                qm = jnp.where(r8 == j, q8[:, h * DH:(h + 1) * DH], 0.0).astype(_BF)
                t = _dot(qm, k_v[h], _NT)
                sg = t if sg is None else sg + t
            sg = sg * scale
            mg = jnp.max(sg, axis=1, keepdims=True)
            pg = jnp.exp(sg - mg)
            ls.append(jnp.sum(pg, axis=1, keepdims=True))
            ps.append(pg.astype(_BF))
            issue(slot4, cuts[g], cuts[g + 1], 8)

        bounds = [0] + list(groups)
        last = bounds[-1]
        assert last == NR - 4

        def issue5(r0, r1):
            for g in range(nG):
                lo, hi = max(r0, bounds[g]), min(r1, bounds[g + 1])
                if lo < hi:
                    issue(slot5(g), lo, hi, peel=1000 if lo else NR)

        issue5(0, sched[0])
        wait_all(v_v, S_V)
        os_ = []
        for g in range(H // 8):
            og = jnp.zeros((8, DH), _F32)
            for j in range(8):
                h = g * 8 + j
                og = jnp.where(r8 == j, _dot(ps[g], v_v[h]), og)
            os_.append(og / ls[g])
        oa = flatten(jnp.concatenate(os_, axis=0))
        issue5(sched[0], sched[1])
        wait_all(wuv_v, S_WUV)
        ob = flatten(contract(wuv_v))
        ocol = {}
        for j in range(NB - vpu_tail, NB):
            row = oa[0:1, (j + 1) * 1024 - 128:(j + 1) * 1024].astype(_F32)
            ocol[j] = jnp.transpose(jnp.broadcast_to(row, (128, 128)))

        acc = [None, None]

        def oproj(which, r0, r1, sem, js=range(NB)):
            w_v, lhs = ((wo_v, oa), (bwo_v, ob))[which]
            js = list(js)
            wait_all(w_v.at[pl.ds(js[0], len(js)), pl.ds(r0, r1 - r0), :], sem)
            for j in js:
                t = _dot(lhs[:, j * 1024 + r0:j * 1024 + r1], w_v[j, r0:r1, :])
                acc[which] = t if acc[which] is None else acc[which] + t

        def grp(which, g):
            oproj(which, bounds[g] * 32, bounds[g + 1] * 32, S_O + which * nG + g)

        S_T = S_O + 2 * nG
        issue5(sched[1], sched[2])
        for g in range(early):
            grp(1, g)
            grp(0, g)
        issue5(sched[2], last)

        def tail_sem(j, i):
            if j == NB - 1 and vpu_tail:
                return S_T + 1 + j + max(0, i - last - 1)
            return S_T + 1 + j
        for j in range(NB):
            for i in range(last, NR):
                wide(wo_hbm, wo_v, j, tail_sem(j, i))(i)[0].start(priority=1)
                wide(bwo_hbm, bwo_v, j, S_T)(i)[0].start(priority=0)
        for g in range(early, nG - 1):
            grp(1, g)
            grp(0, g)
        grp(1, nG - 1)
        oproj(1, last * 32, NR * 32, S_T)
        o_ref[0, :, D:2 * D] = acc[1][0:1, :].astype(o_ref.dtype)
        grp(0, nG - 1)
        for j in range(NB - vpu_tail):
            oproj(0, last * 32, NR * 32, S_T + 1 + j, [j])
        if not vpu_tail:
            o_ref[0, :, 0:D] = acc[0][0:1, :].astype(o_ref.dtype)
            return
        r8w = lax.broadcasted_iota(jnp.int32, (8, D), 0)
        part = jnp.where(r8w == 0, acc[0], 0.0)

        def vpu(j, a, b, sem, part):
            r0 = last * 32
            wait_all(wo_v.at[j, pl.ds(r0 + a, b - a), :], sem)
            w = wo_v[j, r0 + a:r0 + b, :].astype(_F32)
            c = ocol[j][a:b, :]
            prod = w * jnp.concatenate([c] * (D // 128), axis=1)
            for u in range((b - a) // 8):
                part = part + prod[u * 8:(u + 1) * 8, :]
            return part
        for j in range(NB - vpu_tail, NB - 1):
            part = vpu(j, 0, 128, S_T + 1 + j, part)
        j = NB - 1
        part = vpu(j, 0, 64, S_T + 1 + j, part)
        part = vpu(j, 64, 96, S_T + 2 + j, part)
        part = vpu(j, 96, 128, S_T + 3 + j, part)
        o_ref[0, :, 0:D] = jnp.sum(part, axis=0, keepdims=True).astype(o_ref.dtype)

    return kernel


def build(groups=(16, 24, 28), sched=(10, 16, 24), early=1, dA=2, dB=1, prefix=3, vpu_tail=2):
    @jax.jit
    def f(A_x, A_k_cache, A_v_cache, A_wq, A_wo, B_x, B_c_kv, B_w_q, B_w_uk, B_w_uv, B_w_o):
        kernel = _make_kernel(groups, sched, early, dA, dB, prefix, vpu_tail)
        anyspec = pl.BlockSpec(memory_space=pl.ANY)
        scratch = [
            pltpu.VMEM((1, 1, D), _BF), pltpu.VMEM((1, 1, D), _BF),
            pltpu.VMEM((H, W, DH), _BF), pltpu.VMEM((H, W, DH), _BF),
            pltpu.VMEM((NB, D // NB, HD), _BF), pltpu.VMEM((NB, HD // NB, D), _BF),
            pltpu.VMEM((NB, SK // NB, DC), _BF),
            pltpu.VMEM((NB * BLK, DH), _BF), pltpu.VMEM((NB * BLK, DH), _BF),
            pltpu.VMEM((NB * BLK, DH), _BF), pltpu.VMEM((NB, HD // NB, D), _BF),
            pltpu.VMEM((128, BLK), _BF),
            pltpu.VMEM((NB, H, BLK), _BF),
            pltpu.SemaphoreType.DMA((8 + 2 * len(groups) + 7,)),
        ]
        return pl.pallas_call(
            kernel,
            out_shape=jax.ShapeDtypeStruct((1, 1, 2 * D), _BF),
            in_specs=[anyspec] * 11,
            out_specs=pl.BlockSpec(memory_space=pltpu.VMEM),
            scratch_shapes=scratch,
            compiler_params=pltpu.CompilerParams(
                vmem_limit_bytes=96 * 1024 * 1024,
                disable_bounds_checks=True,
                disable_semaphore_checks=True),
        )(A_x, A_k_cache, A_v_cache, A_wq.reshape(NB, D // NB, HD),
          A_wo.reshape(NB, HD // NB, D), B_x, B_c_kv.reshape(NB, SK // NB, DC),
          B_w_q.reshape(NB * BLK, DH), B_w_uk.reshape(NB * BLK, DH),
          B_w_uv.reshape(NB * BLK, DH), B_w_o.reshape(NB, HD // NB, D))
    return f


_impl = build(dA=2,dB=1)


@jax.jit
def pallas_concat_heads__sliding_block_cached__compressed_kv_cla__decode_kernel(
    A_x, A_k_cache, A_v_cache, A_wq, A_wo, B_x, B_c_kv, B_w_q, B_w_uk, B_w_uv, B_w_o,
):
    return _impl(A_x, A_k_cache, A_v_cache, A_wq, A_wo, B_x, B_c_kv, B_w_q, B_w_uk, B_w_uv, B_w_o)
```

```python
import jax
import jax.numpy as jnp
from jax import lax
import jax.experimental.pallas as pl
import jax.experimental.pallas.tpu as pltpu

_NN = (((1,), (0,)), ((), ()))
_NT = (((1,), (1,)), ((), ()))
_BF = jnp.bfloat16
_F32 = jnp.float32

H, DH, SK, W, D, DC = 32, 128, 4096, 1024, 512, 512
HD = H * DH
NB = 4
BLK = 128 * H
NR = 32


def _dot(a, b, dims=_NN):
    return lax.dot_general(a, b, dims, preferred_element_type=_F32)


def _mo(x, m):
    return x if isinstance(x, int) else pl.multiple_of(x, m)


def _make_kernel(groups, sched, early, dA, dB, prefix, vpu_tail):
    scale = DH ** -0.5
    nG = len(groups)

    def kernel(ax_hbm, k_hbm, v_hbm, wq_hbm, wo_hbm, bx_hbm, ckv_hbm, bwq_hbm,
               wuk_hbm, wuv_hbm, bwo_hbm, o_ref,
               ax_v, bx_v, k_v, v_v, wq_v, wo_v, ckv_v, bwq_v, wuk_v, wuv_v,
               bwo_v, rexp_v, exp_v, sems):
        S_X, S_BWQ, S_WQ, S_WUK, S_CKV, S_K, S_V, S_WUV, S_O = range(9)

        def cp(src, dst, sem):
            return pltpu.make_async_copy(src, dst, sems.at[sem])

        def narrow(hbm, vm, j, sem):
            dr = dB * 8

            def mk(i):
                if isinstance(i, int) and i == 0 and j == 0 and dr:
                    a, b = pl.ds(0, 128 - dr), pl.ds(NB * BLK - dr, dr)
                    return [cp(hbm.at[a], vm.at[a], sem), cp(hbm.at[b], vm.at[b], sem)]
                sl = pl.ds(_mo((j * NR + i) * 128 - dr, 8), 128)
                return [cp(hbm.at[sl], vm.at[sl], sem)]
            return mk

        def wide(hbm, vm, j, sem):
            def mk(i):
                sl = pl.ds(_mo(i * 32, 32), 32)
                return [cp(hbm.at[j, sl, :], vm.at[j, sl, :], sem)]
            return mk

        def wq_stream(j):
            def mk(i):
                r = pl.ds(_mo((i >> 1) * 8, 8), 8)
                c = pl.ds(_mo((i & 1) * (HD // 2), HD // 2), HD // 2)
                return [cp(wq_hbm.at[j, r, c], wq_v.at[j, r, c], S_WQ)]
            return mk

        def kv_stream(hbm, vm, s, sem):
            dr = dA * 8

            def mk(i):
                h = 4 * s + (i >> 3)
                if isinstance(i, int) and i % 8 == 0 and dr:
                    return [cp(hbm.at[0, h, pl.ds(SK - W, 128 - dr), :],
                               vm.at[h, pl.ds(0, 128 - dr), :], sem),
                            cp(hbm.at[0, h, pl.ds(SK - dr, dr), :],
                               vm.at[h, pl.ds(W - dr, dr), :], sem)]
                r = _mo((i & 7) * 128 - dr, 8)
                return [cp(hbm.at[0, h, pl.ds(SK - W + r, 128), :],
                           vm.at[h, pl.ds(r, 128), :], sem)]
            return mk

        def interleave(a, b):
            return [x for t in zip(a, b) for x in t]

        def issue(streams, r0, r1, peel=NR, thread=None):
            def one(i):
                for s, mk in enumerate(streams):
                    for c in mk(i):
                        c.start(priority=(s + 1) % 2 if thread is None else thread)

            def body(i, c):
                one(i)
                return c
            i = r0
            while i < r1:
                if i % peel == 0:
                    one(i)
                    i += 1
                    continue
                e = min(r1, (i // peel + 1) * peel)
                lax.fori_loop(i, e, body, 0)
                i = e

        def wait_all(vm, sem):
            pltpu.make_async_copy(vm, vm, sems.at[sem]).wait()

        slot1 = ([narrow(bwq_hbm, bwq_v, j, S_BWQ) for j in range(NB)]
                 + [wq_stream(j) for j in range(NB)]
                 + [narrow(wuk_hbm, wuk_v, j, S_WUK) for j in range(NB)])
        slot2 = []
        for j in range(NB):
            slot2 += [kv_stream(k_hbm, k_v, j, S_K), wide(ckv_hbm, ckv_v, j, S_CKV),
                      kv_stream(k_hbm, k_v, j + 4, S_K)]
        slot3 = ([kv_stream(v_hbm, v_v, s, S_V) for s in range(8)]
                 + [narrow(wuv_hbm, wuv_v, j, S_WUV) for j in range(NB)])

        def slot5(g):
            return interleave([wide(wo_hbm, wo_v, j, S_O + g) for j in (0, 2, 1, 3)],
                              [wide(bwo_hbm, bwo_v, j, S_O + nG + g) for j in (2, 0, 3, 1)])

        c_bx = cp(bx_hbm, bx_v, S_X)
        c_ax = cp(ax_hbm, ax_v, S_X)
        if prefix:
            issue(slot1, 0, prefix, thread=1)
        c_bx.start()
        c_ax.start()
        issue(slot1, prefix, 8)

        def hmask():
            return (lax.broadcasted_iota(jnp.int32, (H, BLK), 1) % H
                    == lax.broadcasted_iota(jnp.int32, (H, BLK), 0))
        r8 = lax.broadcasted_iota(jnp.int32, (8, DH), 0)

        def expand(vals):
            hm = hmask()
            for b in range(NB):
                e = _dot(vals[:, b * 128:(b + 1) * 128], rexp_v[...])
                exp_v[b] = jnp.where(hm, e, 0.0).astype(_BF)

        def contract(w_v):
            acc = _dot(exp_v[0], w_v[0:BLK, :])
            for b in range(1, NB):
                acc += _dot(exp_v[b], w_v[b * BLK:(b + 1) * BLK, :])
            return acc

        def flatten(t):
            parts = []
            for h in range(H):
                g = h // 8
                parts.append(jnp.where(r8 == h % 8, t[g * 8:(g + 1) * 8, :], 0.0))
            flat = jnp.sum(jnp.concatenate(parts, axis=1), axis=0, keepdims=True)
            return jnp.broadcast_to(flat, (8, HD)).astype(_BF)

        rows = lax.broadcasted_iota(jnp.int32, (128, BLK), 0)
        cols = lax.broadcasted_iota(jnp.int32, (128, BLK), 1)
        rexp_v[...] = jnp.where(cols // H == rows, 1.0, 0.0).astype(_BF)
        issue(slot1, 8, 16)
        c_bx.wait()
        c_ax.wait()
        expand(jnp.broadcast_to(bx_v[0], (H, D)))
        issue(slot1, 16, NR)

        issue(slot2, 0, 8, 8)
        wait_all(bwq_v, S_BWQ)
        qb = contract(bwq_v).astype(_BF)
        issue(slot2, 8, 12, 8)
        wait_all(wq_v, S_WQ)
        xa = jnp.broadcast_to(ax_v[0], (8, D))
        q8 = _dot(xa[:, 0:128], wq_v[0])
        for j in range(1, NB):
            q8 += _dot(xa[:, j * 128:(j + 1) * 128], wq_v[j])
        issue(slot2, 12, 16, 8)
        wait_all(wuk_v, S_WUK)
        qa = []
        for b in range(NB):
            z = _dot(qb, wuk_v[b * BLK:(b + 1) * BLK, :], _NT)
            z = jnp.where(hmask(), z, 0.0).astype(_BF)
            qa.append(_dot(z, rexp_v[...], _NT))
            if b == 1:
                issue(slot2, 16, 24, 8)
        qabs = jnp.concatenate(qa, axis=1).astype(_BF)
        issue(slot2, 24, NR, 8)

        issue(slot3, 0, 8, 8)
        wait_all(ckv_v, S_CKV)
        s = jnp.concatenate([_dot(qabs, ckv_v[j], _NT) for j in range(NB)], axis=1) * scale
        m = jnp.max(s, axis=1, keepdims=True)
        p = jnp.exp(s - m)
        l = jnp.sum(p, axis=1, keepdims=True)
        p = p.astype(_BF)
        issue(slot3, 8, 12, 8)
        lat = _dot(p[:, 0:1024], ckv_v[0])
        for j in range(1, NB):
            lat += _dot(p[:, j * 1024:(j + 1) * 1024], ckv_v[j])
        lat = lat / l
        expand(lat.astype(_BF))
        issue(slot3, 12, 16, 8)
        wait_all(k_v, S_K)
        ps = []
        ls = []
        for g in range(H // 8):
            sg = None
            for j in range(8):
                h = g * 8 + j
                qm = jnp.where(r8 == j, q8[:, h * DH:(h + 1) * DH], 0.0).astype(_BF)
                t = _dot(qm, k_v[h], _NT)
                sg = t if sg is None else sg + t
            sg = sg * scale
            mg = jnp.max(sg, axis=1, keepdims=True)
            pg = jnp.exp(sg - mg)
            ls.append(jnp.sum(pg, axis=1, keepdims=True))
            ps.append(pg.astype(_BF))
            if g % 2 == 1:
                issue(slot3, 12 + 4 * g, 20 + 4 * g, 8)

        bounds = [0] + list(groups)
        last = bounds[-1]
        assert last == NR - 4

        def issue5(r0, r1):
            for g in range(nG):
                lo, hi = max(r0, bounds[g]), min(r1, bounds[g + 1])
                if lo < hi:
                    issue(slot5(g), lo, hi, peel=1000 if lo else NR)

        issue5(0, sched[0])
        wait_all(v_v, S_V)
        os_ = []
        for g in range(H // 8):
            og = jnp.zeros((8, DH), _F32)
            for j in range(8):
                h = g * 8 + j
                og = jnp.where(r8 == j, _dot(ps[g], v_v[h]), og)
            os_.append(og / ls[g])
        oa = flatten(jnp.concatenate(os_, axis=0))
        issue5(sched[0], sched[1])
        wait_all(wuv_v, S_WUV)
        ob = flatten(contract(wuv_v))
        ocol = {}
        for j in range(NB - vpu_tail, NB):
            row = oa[0:1, (j + 1) * 1024 - 128:(j + 1) * 1024].astype(_F32)
            ocol[j] = jnp.transpose(jnp.broadcast_to(row, (128, 128)))

        acc = [None, None]

        def oproj(which, r0, r1, sem, js=range(NB)):
            w_v, lhs = ((wo_v, oa), (bwo_v, ob))[which]
            js = list(js)
            wait_all(w_v.at[pl.ds(js[0], len(js)), pl.ds(r0, r1 - r0), :], sem)
            for j in js:
                t = _dot(lhs[:, j * 1024 + r0:j * 1024 + r1], w_v[j, r0:r1, :])
                acc[which] = t if acc[which] is None else acc[which] + t

        def grp(which, g):
            oproj(which, bounds[g] * 32, bounds[g + 1] * 32, S_O + which * nG + g)

        S_T = S_O + 2 * nG
        issue5(sched[1], sched[2])
        for g in range(early):
            grp(1, g)
            grp(0, g)
        issue5(sched[2], last)

        def tail_sem(j, i):
            if j == NB - 1 and vpu_tail:
                return S_T + 1 + j + max(0, i - last - 1)
            return S_T + 1 + j
        for j in range(NB):
            for i in range(last, NR):
                wide(wo_hbm, wo_v, j, tail_sem(j, i))(i)[0].start(priority=1)
                wide(bwo_hbm, bwo_v, j, S_T)(i)[0].start(priority=0)
        for g in range(early, nG - 1):
            grp(1, g)
            grp(0, g)
        grp(1, nG - 1)
        oproj(1, last * 32, NR * 32, S_T)
        o_ref[0, :, D:2 * D] = acc[1][0:1, :].astype(o_ref.dtype)
        grp(0, nG - 1)
        for j in range(NB - vpu_tail):
            oproj(0, last * 32, NR * 32, S_T + 1 + j, [j])
        if not vpu_tail:
            o_ref[0, :, 0:D] = acc[0][0:1, :].astype(o_ref.dtype)
            return
        r8w = lax.broadcasted_iota(jnp.int32, (8, D), 0)
        part = jnp.where(r8w == 0, acc[0], 0.0)

        def vpu(j, a, b, sem, part):
            r0 = last * 32
            wait_all(wo_v.at[j, pl.ds(r0 + a, b - a), :], sem)
            w = wo_v[j, r0 + a:r0 + b, :].astype(_F32)
            c = ocol[j][a:b, :]
            prod = w * jnp.concatenate([c] * (D // 128), axis=1)
            for u in range((b - a) // 8):
                part = part + prod[u * 8:(u + 1) * 8, :]
            return part
        for j in range(NB - vpu_tail, NB - 1):
            part = vpu(j, 0, 128, S_T + 1 + j, part)
        j = NB - 1
        part = vpu(j, 0, 64, S_T + 1 + j, part)
        part = vpu(j, 64, 96, S_T + 2 + j, part)
        part = vpu(j, 96, 128, S_T + 3 + j, part)
        o_ref[0, :, 0:D] = jnp.sum(part, axis=0, keepdims=True).astype(o_ref.dtype)

    return kernel


def build(groups=(16, 24, 28), sched=(10, 16, 24), early=1, dA=2, dB=1, prefix=2, vpu_tail=2):
    @jax.jit
    def f(A_x, A_k_cache, A_v_cache, A_wq, A_wo, B_x, B_c_kv, B_w_q, B_w_uk, B_w_uv, B_w_o):
        kernel = _make_kernel(groups, sched, early, dA, dB, prefix, vpu_tail)
        anyspec = pl.BlockSpec(memory_space=pl.ANY)
        scratch = [
            pltpu.VMEM((1, 1, D), _BF), pltpu.VMEM((1, 1, D), _BF),
            pltpu.VMEM((H, W, DH), _BF), pltpu.VMEM((H, W, DH), _BF),
            pltpu.VMEM((NB, D // NB, HD), _BF), pltpu.VMEM((NB, HD // NB, D), _BF),
            pltpu.VMEM((NB, SK // NB, DC), _BF),
            pltpu.VMEM((NB * BLK, DH), _BF), pltpu.VMEM((NB * BLK, DH), _BF),
            pltpu.VMEM((NB * BLK, DH), _BF), pltpu.VMEM((NB, HD // NB, D), _BF),
            pltpu.VMEM((128, BLK), _BF),
            pltpu.VMEM((NB, H, BLK), _BF),
            pltpu.SemaphoreType.DMA((8 + 2 * len(groups) + 7,)),
        ]
        return pl.pallas_call(
            kernel,
            out_shape=jax.ShapeDtypeStruct((1, 1, 2 * D), _BF),
            in_specs=[anyspec] * 11,
            out_specs=pl.BlockSpec(memory_space=pltpu.VMEM),
            scratch_shapes=scratch,
            compiler_params=pltpu.CompilerParams(
                vmem_limit_bytes=96 * 1024 * 1024,
                disable_bounds_checks=True,
                disable_semaphore_checks=True),
        )(A_x, A_k_cache, A_v_cache, A_wq.reshape(NB, D // NB, HD),
          A_wo.reshape(NB, HD // NB, D), B_x, B_c_kv.reshape(NB, SK // NB, DC),
          B_w_q.reshape(NB * BLK, DH), B_w_uk.reshape(NB * BLK, DH),
          B_w_uv.reshape(NB * BLK, DH), B_w_o.reshape(NB, HD // NB, D))
    return f


_impl = build(sched=(12,18,25))


@jax.jit
def pallas_concat_heads__sliding_block_cached__compressed_kv_cla__decode_kernel(
    A_x, A_k_cache, A_v_cache, A_wq, A_wo, B_x, B_c_kv, B_w_q, B_w_uk, B_w_uv, B_w_o,
):
    return _impl(A_x, A_k_cache, A_v_cache, A_wq, A_wo, B_x, B_c_kv, B_w_q, B_w_uk, B_w_uv, B_w_o)
```

```python
import jax
import jax.numpy as jnp
from jax import lax
import jax.experimental.pallas as pl
import jax.experimental.pallas.tpu as pltpu

_NN = (((1,), (0,)), ((), ()))
_NT = (((1,), (1,)), ((), ()))
_BF = jnp.bfloat16
_F32 = jnp.float32

H, DH, SK, W, D, DC = 32, 128, 4096, 1024, 512, 512
HD = H * DH
NB = 4
BLK = 128 * H
NR = 32
RW = HD // NB

OFF_A, OFF_B = 2, 1

GROUPS = (0, 16, 24, 28)
NG = len(GROUPS) - 1
LAST = GROUPS[-1]
VPU_REGIONS = 2

(S_X, S_BWQ, S_WQ, S_WUK, S_CKV, S_K, S_V, S_WUV, S_O) = range(9)
S_T = S_O + 2 * NG
N_SEMS = S_T + NB + 3


def _dot(a, b, dims=_NN):
    return lax.dot_general(a, b, dims, preferred_element_type=_F32)


def _mo(x, m):
    return x if isinstance(x, int) else pl.multiple_of(x, m)


def _kernel(ax_hbm, k_hbm, v_hbm, wq_hbm, wo_hbm, bx_hbm, ckv_hbm, bwq_hbm,
            wuk_hbm, wuv_hbm, bwo_hbm, o_ref,
            ax_v, bx_v, k_v, v_v, wq_v, wo_v, ckv_v, bwq_v, wuk_v, wuv_v,
            bwo_v, rexp_v, exp_v, sems):
    scale = DH ** -0.5

    def cp(src, dst, sem):
        return pltpu.make_async_copy(src, dst, sems.at[sem])

    def same(hbm, vm, idx, sem):
        return cp(hbm.at[idx], vm.at[idx], sem)

    def wait_all(vm, sem):
        cp(vm, vm, sem).wait()

    def narrow(hbm, vm, j, sem):
        dr = OFF_B * 8

        def mk(i, lo):
            if lo == 0 and j == 0:
                return [same(hbm, vm, (pl.ds(0, 128 - dr),), sem),
                        same(hbm, vm, (pl.ds(NB * BLK - dr, dr),), sem)]
            return [same(hbm, vm, (pl.ds(_mo((j * NR + i) * 128 - dr, 8), 128),), sem)]
        return mk

    def wide(hbm, vm, j, sem):
        def mk(i, lo):
            return [same(hbm, vm, (j, pl.ds(_mo(i * 32, 32), 32)), sem)]
        return mk

    def wq_stream(j):
        def mk(i, lo):
            r = pl.ds(_mo((i >> 1) * 8, 8), 8)
            c = pl.ds(_mo((i & 1) * (HD // 2), HD // 2), HD // 2)
            return [same(wq_hbm, wq_v, (j, r, c), S_WQ)]
        return mk

    def kv_stream(hbm, vm, s, sem):
        dr = OFF_A * 8

        def mk(i, lo):
            h = 4 * s + lo // 8

            def rows(r, n):
                return cp(hbm.at[0, h, pl.ds(SK - W + r, n)], vm.at[h, pl.ds(r, n)], sem)
            if lo % 8 == 0:
                return [rows(0, 128 - dr), rows(W - dr, dr)]
            return [rows(_mo((i - lo // 8 * 8) * 128 - dr, 8), 128)]
        return mk

    def wide2(hbm, vm, j, d, sem0, g):
        cl, cr = pl.ds(0, D - d * 128), pl.ds(D - d * 128, d * 128)

        def mk(i, lo):
            first = lo == GROUPS[g]
            rr = pl.ds(0, 24) if lo == 0 else pl.ds(_mo(i * 32 - 8, 8), 32)
            return [same(hbm, vm, (j, rr, cr), sem0 + g - (1 if first and g else 0)),
                    same(hbm, vm, (j, pl.ds(_mo(i * 32, 32), 32), cl), sem0 + g)]
        return mk

    def issue(streams, r0, r1, static=(0,), thread=None):
        def one(i, lo):
            for s, mk in enumerate(streams):
                for c in mk(i, lo):
                    c.start(priority=(s + 1) % 2 if thread is None else thread)

        i = r0
        while i < r1:
            if i in static:
                one(i, i)
                i += 1
                continue
            e = min([r1] + [t for t in static if t > i])

            def body(t, carry, lo=i):
                one(t, lo)
                return carry
            lax.fori_loop(i, e, body, 0)
            i = e

    heads = (0, 8, 16, 24)
    slot1 = ([narrow(bwq_hbm, bwq_v, j, S_BWQ) for j in range(NB)]
             + [wq_stream(j) for j in range(NB)]
             + [narrow(wuk_hbm, wuk_v, j, S_WUK) for j in range(NB)])
    slot2 = []
    for j in range(NB):
        slot2 += [kv_stream(k_hbm, k_v, j, S_K), wide(ckv_hbm, ckv_v, j, S_CKV),
                  kv_stream(k_hbm, k_v, j + 4, S_K)]
    slot3 = ([kv_stream(v_hbm, v_v, s, S_V) for s in range(8)]
             + [narrow(wuv_hbm, wuv_v, j, S_WUV) for j in range(NB)])

    def issue4(r0, r1):
        for g in range(NG):
            lo, hi = max(r0, GROUPS[g]), min(r1, GROUPS[g + 1])
            if lo < hi:
                streams = []
                for ja, jb in zip((0, 2, 1, 3), (2, 0, 3, 1)):
                    streams += [wide2(wo_hbm, wo_v, ja, OFF_A, S_O, g),
                                wide2(bwo_hbm, bwo_v, jb, OFF_B, S_O + NG, g)]
                issue(streams, lo, hi, static=GROUPS)

    r8 = lax.broadcasted_iota(jnp.int32, (8, DH), 0)

    def hmask():
        return (lax.broadcasted_iota(jnp.int32, (H, BLK), 1) % H
                == lax.broadcasted_iota(jnp.int32, (H, BLK), 0))

    def expand(vals):
        hm = hmask()
        for b in range(NB):
            e = _dot(vals[:, b * 128:(b + 1) * 128], rexp_v[...])
            exp_v[b] = jnp.where(hm, e, 0.0).astype(_BF)

    def contract(w_v):
        acc = _dot(exp_v[0], w_v[0:BLK, :])
        for b in range(1, NB):
            acc += _dot(exp_v[b], w_v[b * BLK:(b + 1) * BLK, :])
        return acc

    def flatten(t):
        parts = [jnp.where(r8 == h % 8, t[h // 8 * 8:h // 8 * 8 + 8, :], 0.0)
                 for h in range(H)]
        flat = jnp.sum(jnp.concatenate(parts, axis=1), axis=0, keepdims=True)
        return jnp.broadcast_to(flat, (8, HD)).astype(_BF)

    c_bx = cp(bx_hbm, bx_v, S_X)
    c_ax = cp(ax_hbm, ax_v, S_X)
    issue(slot1, 0, 2, thread=1)
    c_bx.start()
    c_ax.start()
    issue(slot1, 2, 8)
    rexp_v[...] = jnp.where(
        lax.broadcasted_iota(jnp.int32, (128, BLK), 1) // H
        == lax.broadcasted_iota(jnp.int32, (128, BLK), 0), 1.0, 0.0).astype(_BF)
    issue(slot1, 8, 16)
    c_bx.wait()
    c_ax.wait()
    expand(jnp.broadcast_to(bx_v[0], (H, D)))
    issue(slot1, 16, NR)

    issue(slot2, 0, 8, heads)
    wait_all(bwq_v, S_BWQ)
    qb = contract(bwq_v).astype(_BF)
    issue(slot2, 8, 12, heads)
    wait_all(wq_v, S_WQ)
    xa = jnp.broadcast_to(ax_v[0], (8, D))
    q8 = _dot(xa[:, 0:128], wq_v[0])
    for j in range(1, NB):
        q8 += _dot(xa[:, j * 128:(j + 1) * 128], wq_v[j])
    issue(slot2, 12, 16, heads)
    wait_all(wuk_v, S_WUK)
    qa = []
    for b in range(NB):
        z = _dot(qb, wuk_v[b * BLK:(b + 1) * BLK, :], _NT)
        z = jnp.where(hmask(), z, 0.0).astype(_BF)
        qa.append(_dot(z, rexp_v[...], _NT))
        if b == 1:
            issue(slot2, 16, 24, heads)
    qabs = jnp.concatenate(qa, axis=1).astype(_BF)
    issue(slot2, 24, NR, heads)

    issue(slot3, 0, 8, heads)
    wait_all(ckv_v, S_CKV)
    s = jnp.concatenate([_dot(qabs, ckv_v[j], _NT) for j in range(NB)], axis=1) * scale
    p = jnp.exp(s - jnp.max(s, axis=1, keepdims=True))
    l = jnp.sum(p, axis=1, keepdims=True)
    p = p.astype(_BF)
    issue(slot3, 8, 12, heads)
    lat = _dot(p[:, 0:RW], ckv_v[0])
    for j in range(1, NB):
        lat += _dot(p[:, j * RW:(j + 1) * RW], ckv_v[j])
    expand((lat / l).astype(_BF))
    issue(slot3, 12, 16, heads)
    wait_all(k_v, S_K)
    ps, ls = [], []
    for g in range(H // 8):
        sg = None
        for j in range(8):
            h = g * 8 + j
            qm = jnp.where(r8 == j, q8[:, h * DH:(h + 1) * DH], 0.0).astype(_BF)
            t = _dot(qm, k_v[h], _NT)
            sg = t if sg is None else sg + t
        sg = sg * scale
        pg = jnp.exp(sg - jnp.max(sg, axis=1, keepdims=True))
        ls.append(jnp.sum(pg, axis=1, keepdims=True))
        ps.append(pg.astype(_BF))
        if g % 2 == 1:
            issue(slot3, 12 + 4 * g, 20 + 4 * g, heads)

    issue4(0, 10)
    wait_all(v_v, S_V)
    os_ = []
    for g in range(H // 8):
        og = jnp.zeros((8, DH), _F32)
        for j in range(8):
            og = jnp.where(r8 == j, _dot(ps[g], v_v[g * 8 + j]), og)
        os_.append(og / ls[g])
        if g == 1:
            issue4(10, 13)
    oa = flatten(jnp.concatenate(os_, axis=0))
    issue4(13, 16)
    wait_all(wuv_v, S_WUV)
    ob = flatten(contract(wuv_v))
    ocol = {}
    for j in range(NB - VPU_REGIONS, NB):
        row = oa[0:1, (j + 1) * RW - 128:(j + 1) * RW].astype(_F32)
        ocol[j] = jnp.transpose(jnp.broadcast_to(row, (128, 128)))

    proj = ((wo_hbm, wo_v, oa, OFF_A), (bwo_hbm, bwo_v, ob, OFF_B))
    acc = [None, None]

    def accumulate(which, r0, r1, js):
        _, w_v, lhs, _ = proj[which]
        for j in js:
            t = _dot(lhs[:, j * RW + r0:j * RW + r1], w_v[j, r0:r1, :])
            acc[which] = t if acc[which] is None else acc[which] + t

    def group(which, g):
        _, w_v, _, d = proj[which]
        r0, r1 = GROUPS[g] * 32, GROUPS[g + 1] * 32
        q0, q1 = (r0 + 24 if g else 0), min(r1 + 24, LAST * 32)
        sem = S_O + which * NG + g
        wait_all(w_v.at[:, pl.ds(r0, r1 - r0), pl.ds(0, D - d * 128)], sem)
        wait_all(w_v.at[:, pl.ds(q0, q1 - q0), pl.ds(D - d * 128, d * 128)], sem)
        accumulate(which, r0, r1, range(NB))

    issue4(16, 24)
    group(1, 0)
    group(0, 0)
    issue4(24, LAST)
    for j in range(NB):
        for which in (1, 0):
            hbm, w_v, _, d = proj[which]
            idx = (j, pl.ds(LAST * 32 - 8, 8), pl.ds(D - d * 128, d * 128))
            same(hbm, w_v, idx, S_O + which * NG + NG - 1).start(priority=1 - which)
    for j in range(NB):
        for i in range(LAST, NR):
            sem = S_T + 1 + j + (max(0, i - LAST - 1) if j == NB - 1 else 0)
            same(wo_hbm, wo_v, (j, pl.ds(i * 32, 32)), sem).start(priority=1)
            same(bwo_hbm, bwo_v, (j, pl.ds(i * 32, 32)), S_T).start(priority=0)
    for g in range(1, NG - 1):
        group(1, g)
        group(0, g)
    T0 = LAST * 32
    group(1, NG - 1)
    wait_all(bwo_v.at[:, pl.ds(T0, RW - T0)], S_T)
    accumulate(1, T0, RW, range(NB))
    o_ref[0, :, D:2 * D] = acc[1][0:1, :].astype(o_ref.dtype)
    group(0, NG - 1)
    for j in range(NB - VPU_REGIONS):
        wait_all(wo_v.at[j, pl.ds(T0, RW - T0)], S_T + 1 + j)
        accumulate(0, T0, RW, [j])

    part = jnp.where(lax.broadcasted_iota(jnp.int32, (8, D), 0) == 0, acc[0], 0.0)

    def vpu(j, a, b, sem, part):
        wait_all(wo_v.at[j, pl.ds(T0 + a, b - a)], sem)
        w = wo_v[j, T0 + a:T0 + b, :].astype(_F32)
        prod = w * jnp.concatenate([ocol[j][a:b, :]] * (D // 128), axis=1)
        for u in range((b - a) // 8):
            part = part + prod[u * 8:(u + 1) * 8, :]
        return part

    for j in range(NB - VPU_REGIONS, NB - 1):
        part = vpu(j, 0, 128, S_T + 1 + j, part)
    part = vpu(NB - 1, 0, 64, S_T + NB, part)
    part = vpu(NB - 1, 64, 96, S_T + NB + 1, part)
    part = vpu(NB - 1, 96, 128, S_T + NB + 2, part)
    o_ref[0, :, 0:D] = jnp.sum(part, axis=0, keepdims=True).astype(o_ref.dtype)


def _compiler_params():
    kw = dict(vmem_limit_bytes=96 * 1024 * 1024)
    for name in ("disable_bounds_checks", "disable_semaphore_checks"):
        if hasattr(pltpu.CompilerParams, name):
            kw[name] = True
    return pltpu.CompilerParams(**kw)


@jax.jit
def pallas_concat_heads__sliding_block_cached__compressed_kv_cla__decode_kernel(
    A_x: jax.Array,
    A_k_cache: jax.Array,
    A_v_cache: jax.Array,
    A_wq: jax.Array,
    A_wo: jax.Array,
    B_x: jax.Array,
    B_c_kv: jax.Array,
    B_w_q: jax.Array,
    B_w_uk: jax.Array,
    B_w_uv: jax.Array,
    B_w_o: jax.Array,
):
    assert A_x.shape == (1, 1, D) and B_x.shape == (1, 1, D)
    assert A_k_cache.shape == (1, H, SK, DH) and A_v_cache.shape == (1, H, SK, DH)
    assert B_c_kv.shape == (1, SK, DC) and W == min(4096, max(256, SK // 4))
    anyspec = pl.BlockSpec(memory_space=pl.ANY)
    scratch = [
        pltpu.VMEM((1, 1, D), _BF), pltpu.VMEM((1, 1, D), _BF),
        pltpu.VMEM((H, W, DH), _BF), pltpu.VMEM((H, W, DH), _BF),
        pltpu.VMEM((NB, D // NB, HD), _BF), pltpu.VMEM((NB, RW, D), _BF),
        pltpu.VMEM((NB, SK // NB, DC), _BF),
        pltpu.VMEM((NB * BLK, DH), _BF), pltpu.VMEM((NB * BLK, DH), _BF),
        pltpu.VMEM((NB * BLK, DH), _BF), pltpu.VMEM((NB, RW, D), _BF),
        pltpu.VMEM((128, BLK), _BF),
        pltpu.VMEM((NB, H, BLK), _BF),
        pltpu.SemaphoreType.DMA((N_SEMS,)),
    ]
    return pl.pallas_call(
        _kernel,
        out_shape=jax.ShapeDtypeStruct((1, 1, 2 * D), A_x.dtype),
        in_specs=[anyspec] * 11,
        out_specs=pl.BlockSpec(memory_space=pltpu.VMEM),
        scratch_shapes=scratch,
        compiler_params=_compiler_params(),
    )(A_x, A_k_cache, A_v_cache, A_wq.reshape(NB, D // NB, HD),
      A_wo.reshape(NB, RW, D), B_x, B_c_kv.reshape(NB, SK // NB, DC),
      B_w_q.reshape(NB * BLK, DH), B_w_uk.reshape(NB * BLK, DH),
      B_w_uv.reshape(NB * BLK, DH), B_w_o.reshape(NB, RW, D))
```

```python
import jax
import jax.numpy as jnp
from jax import lax
import jax.experimental.pallas as pl
import jax.experimental.pallas.tpu as pltpu

_NN = (((1,), (0,)), ((), ()))
_NT = (((1,), (1,)), ((), ()))
_BF = jnp.bfloat16
_F32 = jnp.float32

H, DH, SK, W, D, DC = 32, 128, 4096, 1024, 512, 512
HD = H * DH
NB = 4
BLK = 128 * H
NR = 32
RW = HD // NB

OFF_A, OFF_B = 2, 1

GROUPS = (0, 16, 24, 28)
NG = len(GROUPS) - 1
LAST = GROUPS[-1]
VPU_REGIONS = 2

(S_X, S_BWQ, S_WQ, S_WUK, S_CKV, S_K, S_V, S_WUV, S_O) = range(9)
S_T = S_O + 2 * NG
N_SEMS = S_T + NB + 3


def _dot(a, b, dims=_NN):
    return lax.dot_general(a, b, dims, preferred_element_type=_F32)


def _mo(x, m):
    return x if isinstance(x, int) else pl.multiple_of(x, m)


def _kernel(*refs):
    pl.run_scoped(lambda sems: _body(*refs, sems), pltpu.SemaphoreType.DMA((N_SEMS,)))


def _body(ax_hbm, k_hbm, v_hbm, wq_hbm, wo_hbm, bx_hbm, ckv_hbm, bwq_hbm,
          wuk_hbm, wuv_hbm, bwo_hbm, o_ref,
          ax_v, bx_v, k_v, v_v, wq_v, wo_v, ckv_v, bwq_v, wuk_v, wuv_v,
          bwo_v, rexp_v, exp_v, sems):
    scale = DH ** -0.5

    def cp(src, dst, sem):
        return pltpu.make_async_copy(src, dst, sems.at[sem])

    def same(hbm, vm, idx, sem):
        return cp(hbm.at[idx], vm.at[idx], sem)

    def wait_all(vm, sem):
        cp(vm, vm, sem).wait()

    def narrow(hbm, vm, j, sem):
        dr = OFF_B * 8

        def mk(i, lo):
            if lo == 0 and j == 0:
                return [same(hbm, vm, (pl.ds(0, 128 - dr),), sem),
                        same(hbm, vm, (pl.ds(NB * BLK - dr, dr),), sem)]
            return [same(hbm, vm, (pl.ds(_mo((j * NR + i) * 128 - dr, 8), 128),), sem)]
        return mk

    def wide(hbm, vm, j, sem):
        def mk(i, lo):
            return [same(hbm, vm, (j, pl.ds(_mo(i * 32, 32), 32)), sem)]
        return mk

    def wq_stream(j):
        def mk(i, lo):
            r = pl.ds(_mo((i >> 1) * 8, 8), 8)
            c = pl.ds(_mo((i & 1) * (HD // 2), HD // 2), HD // 2)
            return [same(wq_hbm, wq_v, (j, r, c), S_WQ)]
        return mk

    def kv_stream(hbm, vm, s, sem):
        dr = OFF_A * 8

        def mk(i, lo):
            h = 4 * s + lo // 8

            def rows(r, n):
                return cp(hbm.at[0, h, pl.ds(SK - W + r, n)], vm.at[h, pl.ds(r, n)], sem)
            if lo % 8 == 0:
                return [rows(0, 128 - dr), rows(W - dr, dr)]
            return [rows(_mo((i - lo // 8 * 8) * 128 - dr, 8), 128)]
        return mk

    def wide2(hbm, vm, j, d, sem0, g):
        cl, cr = pl.ds(0, D - d * 128), pl.ds(D - d * 128, d * 128)

        def mk(i, lo):
            first = lo == GROUPS[g]
            rr = pl.ds(0, 24) if lo == 0 else pl.ds(_mo(i * 32 - 8, 8), 32)
            return [same(hbm, vm, (j, rr, cr), sem0 + g - (1 if first and g else 0)),
                    same(hbm, vm, (j, pl.ds(_mo(i * 32, 32), 32), cl), sem0 + g)]
        return mk

    def issue(streams, r0, r1, static=(0,), thread=None):
        def one(i, lo):
            for s, mk in enumerate(streams):
                for c in mk(i, lo):
                    c.start(priority=(s + 1) % 2 if thread is None else thread)

        i = r0
        while i < r1:
            if i in static:
                one(i, i)
                i += 1
                continue
            e = min([r1] + [t for t in static if t > i])

            def body(t, carry, lo=i):
                one(t, lo)
                return carry
            lax.fori_loop(i, e, body, 0)
            i = e

    heads = (0, 8, 16, 24)
    slot1 = ([narrow(bwq_hbm, bwq_v, j, S_BWQ) for j in range(NB)]
             + [wq_stream(j) for j in range(NB)]
             + [narrow(wuk_hbm, wuk_v, j, S_WUK) for j in range(NB)])
    slot2 = []
    for j in range(NB):
        slot2 += [kv_stream(k_hbm, k_v, j, S_K), wide(ckv_hbm, ckv_v, j, S_CKV),
                  kv_stream(k_hbm, k_v, j + 4, S_K)]
    slot3 = ([kv_stream(v_hbm, v_v, s, S_V) for s in range(8)]
             + [narrow(wuv_hbm, wuv_v, j, S_WUV) for j in range(NB)])

    def issue4(r0, r1):
        for g in range(NG):
            lo, hi = max(r0, GROUPS[g]), min(r1, GROUPS[g + 1])
            if lo < hi:
                streams = []
                for ja, jb in zip((0, 2, 1, 3), (2, 0, 3, 1)):
                    streams += [wide2(wo_hbm, wo_v, ja, OFF_A, S_O, g),
                                wide2(bwo_hbm, bwo_v, jb, OFF_B, S_O + NG, g)]
                issue(streams, lo, hi, static=GROUPS)

    r8 = lax.broadcasted_iota(jnp.int32, (8, DH), 0)

    def hmask():
        return (lax.broadcasted_iota(jnp.int32, (H, BLK), 1) % H
                == lax.broadcasted_iota(jnp.int32, (H, BLK), 0))

    def expand(vals):
        hm = hmask()
        for b in range(NB):
            e = _dot(vals[:, b * 128:(b + 1) * 128], rexp_v[...])
            exp_v[b] = jnp.where(hm, e, 0.0).astype(_BF)

    def contract(w_v):
        acc = _dot(exp_v[0], w_v[0:BLK, :])
        for b in range(1, NB):
            acc += _dot(exp_v[b], w_v[b * BLK:(b + 1) * BLK, :])
        return acc

    def flatten(t):
        parts = [jnp.where(r8 == h % 8, t[h // 8 * 8:h // 8 * 8 + 8, :], 0.0)
                 for h in range(H)]
        flat = jnp.sum(jnp.concatenate(parts, axis=1), axis=0, keepdims=True)
        return jnp.broadcast_to(flat, (8, HD)).astype(_BF)

    c_bx = cp(bx_hbm, bx_v, S_X)
    c_ax = cp(ax_hbm, ax_v, S_X)
    issue(slot1, 0, 2, thread=1)
    c_bx.start()
    c_ax.start()
    issue(slot1, 2, 8)
    rexp_v[...] = jnp.where(
        lax.broadcasted_iota(jnp.int32, (128, BLK), 1) // H
        == lax.broadcasted_iota(jnp.int32, (128, BLK), 0), 1.0, 0.0).astype(_BF)
    issue(slot1, 8, 16)
    c_bx.wait()
    c_ax.wait()
    expand(jnp.broadcast_to(bx_v[0], (H, D)))
    issue(slot1, 16, NR)

    issue(slot2, 0, 8, heads)
    wait_all(bwq_v, S_BWQ)
    qb = contract(bwq_v).astype(_BF)
    issue(slot2, 8, 12, heads)
    wait_all(wq_v, S_WQ)
    xa = jnp.broadcast_to(ax_v[0], (8, D))
    q8 = _dot(xa[:, 0:128], wq_v[0])
    for j in range(1, NB):
        q8 += _dot(xa[:, j * 128:(j + 1) * 128], wq_v[j])
    issue(slot2, 12, 16, heads)
    wait_all(wuk_v, S_WUK)
    qa = []
    for b in range(NB):
        z = _dot(qb, wuk_v[b * BLK:(b + 1) * BLK, :], _NT)
        z = jnp.where(hmask(), z, 0.0).astype(_BF)
        qa.append(_dot(z, rexp_v[...], _NT))
        if b == 1:
            issue(slot2, 16, 24, heads)
    qabs = jnp.concatenate(qa, axis=1).astype(_BF)
    issue(slot2, 24, NR, heads)

    issue(slot3, 0, 8, heads)
    wait_all(ckv_v, S_CKV)
    s = jnp.concatenate([_dot(qabs, ckv_v[j], _NT) for j in range(NB)], axis=1) * scale
    p = jnp.exp(s - jnp.max(s, axis=1, keepdims=True))
    l = jnp.sum(p, axis=1, keepdims=True)
    p = p.astype(_BF)
    issue(slot3, 8, 12, heads)
    lat = _dot(p[:, 0:RW], ckv_v[0])
    for j in range(1, NB):
        lat += _dot(p[:, j * RW:(j + 1) * RW], ckv_v[j])
    expand((lat / l).astype(_BF))
    issue(slot3, 12, 16, heads)
    wait_all(k_v, S_K)
    ps, ls = [], []
    for g in range(H // 8):
        sg = None
        for j in range(8):
            h = g * 8 + j
            qm = jnp.where(r8 == j, q8[:, h * DH:(h + 1) * DH], 0.0).astype(_BF)
            t = _dot(qm, k_v[h], _NT)
            sg = t if sg is None else sg + t
        sg = sg * scale
        pg = jnp.exp(sg - jnp.max(sg, axis=1, keepdims=True))
        ls.append(jnp.sum(pg, axis=1, keepdims=True))
        ps.append(pg.astype(_BF))
        if g % 2 == 1:
            issue(slot3, 12 + 4 * g, 20 + 4 * g, heads)

    issue4(0, 10)
    wait_all(v_v, S_V)
    os_ = []
    for g in range(H // 8):
        og = jnp.zeros((8, DH), _F32)
        for j in range(8):
            og = jnp.where(r8 == j, _dot(ps[g], v_v[g * 8 + j]), og)
        os_.append(og / ls[g])
        if g == 1:
            issue4(10, 13)
    oa = flatten(jnp.concatenate(os_, axis=0))
    issue4(13, 16)
    wait_all(wuv_v, S_WUV)
    ob = flatten(contract(wuv_v))
    ocol = {}
    for j in range(NB - VPU_REGIONS, NB):
        row = oa[0:1, (j + 1) * RW - 128:(j + 1) * RW].astype(_F32)
        ocol[j] = jnp.transpose(jnp.broadcast_to(row, (128, 128)))

    proj = ((wo_hbm, wo_v, oa, OFF_A), (bwo_hbm, bwo_v, ob, OFF_B))
    acc = [None, None]

    def accumulate(which, r0, r1, js):
        _, w_v, lhs, _ = proj[which]
        for j in js:
            t = _dot(lhs[:, j * RW + r0:j * RW + r1], w_v[j, r0:r1, :])
            acc[which] = t if acc[which] is None else acc[which] + t

    def group(which, g):
        _, w_v, _, d = proj[which]
        r0, r1 = GROUPS[g] * 32, GROUPS[g + 1] * 32
        q0, q1 = (r0 + 24 if g else 0), min(r1 + 24, LAST * 32)
        sem = S_O + which * NG + g
        wait_all(w_v.at[:, pl.ds(r0, r1 - r0), pl.ds(0, D - d * 128)], sem)
        wait_all(w_v.at[:, pl.ds(q0, q1 - q0), pl.ds(D - d * 128, d * 128)], sem)
        accumulate(which, r0, r1, range(NB))

    issue4(16, 24)
    group(1, 0)
    group(0, 0)
    issue4(24, LAST)
    for j in range(NB):
        for which in (1, 0):
            hbm, w_v, _, d = proj[which]
            idx = (j, pl.ds(LAST * 32 - 8, 8), pl.ds(D - d * 128, d * 128))
            same(hbm, w_v, idx, S_O + which * NG + NG - 1).start(priority=1 - which)
    for j in range(NB):
        for i in range(LAST, NR):
            sem = S_T + 1 + j + (max(0, i - LAST - 1) if j == NB - 1 else 0)
            same(wo_hbm, wo_v, (j, pl.ds(i * 32, 32)), sem).start(priority=1)
            same(bwo_hbm, bwo_v, (j, pl.ds(i * 32, 32)), S_T).start(priority=0)
    for g in range(1, NG - 1):
        group(1, g)
        group(0, g)
    T0 = LAST * 32
    group(1, NG - 1)
    wait_all(bwo_v.at[:, pl.ds(T0, RW - T0)], S_T)
    accumulate(1, T0, RW, range(NB))
    o_ref[0, :, D:2 * D] = acc[1][0:1, :].astype(o_ref.dtype)
    group(0, NG - 1)
    for j in range(NB - VPU_REGIONS):
        wait_all(wo_v.at[j, pl.ds(T0, RW - T0)], S_T + 1 + j)
        accumulate(0, T0, RW, [j])

    part = jnp.where(lax.broadcasted_iota(jnp.int32, (8, D), 0) == 0, acc[0], 0.0)

    def vpu(j, a, b, sem, part):
        wait_all(wo_v.at[j, pl.ds(T0 + a, b - a)], sem)
        w = wo_v[j, T0 + a:T0 + b, :].astype(_F32)
        prod = w * jnp.concatenate([ocol[j][a:b, :]] * (D // 128), axis=1)
        for u in range((b - a) // 8):
            part = part + prod[u * 8:(u + 1) * 8, :]
        return part

    for j in range(NB - VPU_REGIONS, NB - 1):
        part = vpu(j, 0, 128, S_T + 1 + j, part)
    part = vpu(NB - 1, 0, 64, S_T + NB, part)
    part = vpu(NB - 1, 64, 96, S_T + NB + 1, part)
    part = vpu(NB - 1, 96, 128, S_T + NB + 2, part)
    o_ref[0, :, 0:D] = jnp.sum(part, axis=0, keepdims=True).astype(o_ref.dtype)


@jax.jit
def pallas_concat_heads__sliding_block_cached__compressed_kv_cla__decode_kernel(
    A_x: jax.Array,
    A_k_cache: jax.Array,
    A_v_cache: jax.Array,
    A_wq: jax.Array,
    A_wo: jax.Array,
    B_x: jax.Array,
    B_c_kv: jax.Array,
    B_w_q: jax.Array,
    B_w_uk: jax.Array,
    B_w_uv: jax.Array,
    B_w_o: jax.Array,
):
    assert A_x.shape == (1, 1, D) and B_x.shape == (1, 1, D)
    assert A_k_cache.shape == (1, H, SK, DH) and A_v_cache.shape == (1, H, SK, DH)
    assert B_c_kv.shape == (1, SK, DC) and W == min(4096, max(256, SK // 4))
    anyspec = pl.BlockSpec(memory_space=pl.ANY)
    scratch = [
        pltpu.VMEM((1, 1, D), _BF), pltpu.VMEM((1, 1, D), _BF),
        pltpu.VMEM((H, W, DH), _BF), pltpu.VMEM((H, W, DH), _BF),
        pltpu.VMEM((NB, D // NB, HD), _BF), pltpu.VMEM((NB, RW, D), _BF),
        pltpu.VMEM((NB, SK // NB, DC), _BF),
        pltpu.VMEM((NB * BLK, DH), _BF), pltpu.VMEM((NB * BLK, DH), _BF),
        pltpu.VMEM((NB * BLK, DH), _BF), pltpu.VMEM((NB, RW, D), _BF),
        pltpu.VMEM((128, BLK), _BF),
        pltpu.VMEM((NB, H, BLK), _BF),
    ]
    return pl.pallas_call(
        _kernel,
        out_shape=jax.ShapeDtypeStruct((1, 1, 2 * D), A_x.dtype),
        in_specs=[anyspec] * 11,
        out_specs=pl.BlockSpec(memory_space=pltpu.VMEM),
        scratch_shapes=scratch,
        compiler_params=pltpu.CompilerParams(vmem_limit_bytes=96 * 1024 * 1024),
    )(A_x, A_k_cache, A_v_cache, A_wq.reshape(NB, D // NB, HD),
      A_wo.reshape(NB, RW, D), B_x, B_c_kv.reshape(NB, SK // NB, DC),
      B_w_q.reshape(NB * BLK, DH), B_w_uk.reshape(NB * BLK, DH),
      B_w_uv.reshape(NB * BLK, DH), B_w_o.reshape(NB, RW, D))
```
